```python
import jax
import jax.numpy as jnp

def _softmax(x, axis=-1):
    return jax.nn.softmax(x, axis=axis)
def _gelu(x):
    return jax.nn.gelu(x, approximate=True)
def _silu(x):
    return jax.nn.silu(x)
def _sigmoid(x):
    return jax.nn.sigmoid(x)
def _layernorm(x, axis=-1, eps=1e-5):
    m = jnp.mean(x, axis=axis, keepdims=True)
    v = jnp.var(x, axis=axis, keepdims=True)
    return (x - m) / jnp.sqrt(v + eps)
def _scatter_add(tgt, idx, src, axis=0):
    return tgt.at[idx].add(src)
def _segment_sum(src, seg, n):
    return jax.ops.segment_sum(src, seg, n)
class _Rng:
    def __init__(self, key):
        self._k = key
    def _next(self):
        self._k, sub = jax.random.split(self._k)
        return sub
    def normal(self, shape):
        return jax.random.normal(self._next(), shape, dtype=jnp.bfloat16)
    def randint(self, lo, hi, shape):
        return jax.random.randint(self._next(), shape, lo, hi, dtype=jnp.int32)
    def uniform(self, shape, lo=0.0, hi=1.0):
        return jax.random.uniform(self._next(), shape, jnp.bfloat16, lo, hi)
    def permutation(self, n):
        return jax.random.permutation(self._next(), n)


kernel_name = 'gated_mix__sliding_block_cached__dense_activation_gelu__decode'

def setup_inputs():
    _rng = _Rng(jax.random.key(int.from_bytes(__import__("os").urandom(4), "little")))
    _w = (lambda a: (lambda t: t.astype(jnp.bfloat16) if jnp.issubdtype(t.dtype, jnp.floating) else t)(jnp.asarray(a)))
    def _A_setup():
        B, Sq, D = 1, 1, 640
        Hq, Hkv, Sk, Dh = 32, 32, 32768, 192
        assert Hq % Hkv == 0, (Hq, Hkv)
        return {
            "x": _w((lambda *s: _rng.normal(s) * 0.05)(B, Sq, D)),
            "k_cache": _w((lambda *s: _rng.normal(s) * 0.05)(B, Hkv, Sk, Dh)),
            "v_cache": _w((lambda *s: _rng.normal(s) * 0.05)(B, Hkv, Sk, Dh)),
            "wq": _w((lambda *s: _rng.normal(s) * 0.05)(D, Hq * Dh) * (D ** -0.5)),
            "wo": _w((lambda *s: _rng.normal(s) * 0.05)(Hq * Dh, D) * ((Hq * Dh) ** -0.5)),
        }
    _A_in = _A_setup()

    def _B_setup():
        B, S, D, F = 1, 1, 640, 1536
        return {
            "x": _w((lambda *s: _rng.normal(s) * 0.05)(B, S, D)),
            "w1": _w((lambda *s: _rng.normal(s) * 0.05)(D, F) * (D ** -0.5)),
            "b1": _w((lambda *s: _rng.normal(s) * 0.05)(F) * 0.01),
            "w2": _w((lambda *s: _rng.normal(s) * 0.05)(F, D) * (F ** -0.5)),
            "b2": _w((lambda *s: _rng.normal(s) * 0.05)(D) * 0.01),
        }
    _B_in = _B_setup()

    return {
        "A_x": _A_in["x"],
        "A_k_cache": _A_in["k_cache"],
        "A_v_cache": _A_in["v_cache"],
        "A_wq": _A_in["wq"],
        "A_wo": _A_in["wo"],
        "B_x": _B_in["x"],
        "B_w1": _B_in["w1"],
        "B_b1": _B_in["b1"],
        "B_w2": _B_in["w2"],
        "B_b2": _B_in["b2"],
        "gate_w": _w((lambda *s: _rng.normal(s) * 0.05)(640)),
    }

def reference(A_x, A_k_cache, A_v_cache, A_wq, A_wo, B_x, B_w1, B_b1, B_w2, B_b2, gate_w):
    def _A_ref(x, k_cache, v_cache, wq, wo):
        B, Sq, D = x.shape
        Hq, Dh = 32, 192
        Hkv, Sk = k_cache.shape[1], k_cache.shape[2]
        W = min(4096, max(256, Sk // 4))
        rep = Hq // Hkv
        q = (lambda x, *d: x.transpose(*d))((x @ wq).reshape(B, Sq, Hq, Dh), 0, 2, 1, 3)
        k = jnp.repeat(k_cache[:, :, Sk - W:, :], rep, axis=1)
        v = jnp.repeat(v_cache[:, :, Sk - W:, :], rep, axis=1)
        scores = jnp.einsum("bhqd,bhkd->bhqk", q, k) * (Dh ** -0.5)
        p = _softmax(scores, axis=-1)
        o = jnp.einsum("bhqk,bhkd->bhqd", p, v)
        return (lambda x, *d: x.transpose(*d))(o, 0, 2, 1, 3).reshape(B, Sq, Hq * Dh) @ wo

    def _B_ref(x, w1, b1, w2, b2):
        h = jnp.einsum("bsd,df->bsf", x, w1) + b1
        h = _gelu(h)
        return jnp.einsum("bsf,fd->bsd", h, w2) + b2

    x = A_x
    g = _sigmoid((x * gate_w).sum(-1, keepdims=True))
    a = _A_ref(x, A_k_cache, A_v_cache, A_wq, A_wo)
    b = _B_ref(x, B_w1, B_b1, B_w2, B_b2)
    return g * a + (1 - g) * b
```

```python
import jax
import jax.numpy as jnp
from jax import lax
from jax.experimental import pallas as pl
from jax.experimental.pallas import tpu as pltpu

_G = 8
_RC = 128
_LOOKAHEAD = 3
_W2_PIECES = 4


def _make_kernel(H, DH, S, W, D, F):
    G, RC, L, NP = _G, _RC, _LOOKAHEAD, _W2_PIECES
    NG = H // G
    GR = G * DH
    NC = GR // RC
    NCH = NG * 2 * NC
    NBUF = L + 1
    W2R = F // NP
    f32, bf16 = jnp.float32, jnp.bfloat16

    def kernel(x_hbm, k_hbm, v_hbm, wq_hbm, wo_hbm, w1_hbm, b1_hbm, w2_hbm, b2_hbm, gw_hbm,
               o_ref,
               x_v, b1_v, b2_v, gw_v, wq_v, wo_v, w1_v, w2_v, ring, qbd, p_v,
               sem_small, sem_wq, sem_wo, sem_w1, sem_w2, sem_ring):
        def cp_wq(g):
            return pltpu.make_async_copy(wq_hbm.at[:, pl.ds(g * GR, GR)], wq_v.at[g], sem_wq.at[g])

        def cp_wo(g):
            return pltpu.make_async_copy(wo_hbm.at[pl.ds(g * GR, GR), :], wo_v.at[g], sem_wo.at[g])

        def cp_w2(i):
            rows = pl.ds(i * W2R, W2R)
            return pltpu.make_async_copy(w2_hbm.at[rows, :], w2_v.at[rows, :], sem_w2.at[i])

        cp_w1 = pltpu.make_async_copy(w1_hbm, w1_v, sem_w1)
        cp_x = pltpu.make_async_copy(x_hbm, x_v, sem_small.at[0])
        cp_gw = pltpu.make_async_copy(gw_hbm, gw_v, sem_small.at[1])
        cp_b1 = pltpu.make_async_copy(b1_hbm, b1_v, sem_small.at[2])
        cp_b2 = pltpu.make_async_copy(b2_hbm, b2_v, sem_small.at[3])

        def ring_copy(src, row0, slot):
            return pltpu.make_async_copy(
                src.at[pl.ds(row0, RC), pl.ds(S - W, W)], ring.at[slot], sem_ring.at[slot])

        def issue(j):
            g, r = j // (2 * NC), j % (2 * NC)
            is_v, c = r // NC, r % NC
            slot = j % NBUF
            if isinstance(j, int):
                ring_copy(v_hbm if is_v else k_hbm, g * GR + c * RC, slot).start()
            else:
                row0 = pl.multiple_of(g * GR + c * RC, RC)

                @pl.when(is_v == 0)
                def _():
                    ring_copy(k_hbm, row0, slot).start()

                @pl.when(is_v == 1)
                def _():
                    ring_copy(v_hbm, row0, slot).start()

        def advance(i):
            slot = i % NBUF
            ring_copy(k_hbm, 0, slot).wait()
            j = i + L

            @pl.when(j < NCH)
            def _():
                issue(j)

            @pl.when(j == NCH)
            def _():
                cp_w1.start()
                for t in range(NP):
                    cp_w2(t).start()

            return slot

        cp_x.start()
        cp_wq(0).start()
        for j in range(L):
            issue(j)
        cp_gw.start()
        cp_b1.start()
        cp_b2.start()
        for g in range(1, NG):
            cp_wq(g).start()
        cp_x.wait()

        x8 = jnp.broadcast_to(x_v[...].astype(f32), (8, D)).astype(bf16)
        row = lax.broadcasted_iota(jnp.int32, (G, RC), 0)
        col = lax.broadcasted_iota(jnp.int32, (G, RC), 1)

        def group(g, out_acc):
            cp_wo(g).start()
            cp_wq(g).wait()
            q = jnp.dot(x8, wq_v[g], preferred_element_type=f32)
            for c in range(NC):
                own = row == (c * RC + col) // DH
                qbd[c] = jnp.where(own, q[:, c * RC:(c + 1) * RC], 0.0).astype(bf16)

            def kstep(c, s):
                slot = advance(g * 2 * NC + c)
                return s + jnp.dot(qbd[c], ring[slot], preferred_element_type=f32)

            s = lax.fori_loop(0, NC, kstep, jnp.zeros((G, W), f32)) * (DH ** -0.5)
            p = jnp.exp(s - jnp.max(s, axis=1, keepdims=True))
            linv = 1.0 / jnp.sum(p, axis=1, keepdims=True)
            p_v[...] = p.astype(bf16)
            cp_wo(g).wait()

            def vstep(c, acc):
                slot = advance(g * 2 * NC + NC + c)
                o = lax.dot_general(p_v[...], ring[slot], (((1,), (1,)), ((), ())),
                                    preferred_element_type=f32)
                own = row == (c * RC + col) // DH
                o = jnp.where(own, o * linv, 0.0).astype(bf16)
                r0 = pl.multiple_of(c * RC, RC)
                return acc + jnp.dot(o, wo_v[g, pl.ds(r0, RC), :], preferred_element_type=f32)

            return lax.fori_loop(0, NC, vstep, out_acc)

        out_acc = lax.fori_loop(0, NG, group, jnp.zeros((G, D), f32))
        a = jnp.sum(out_acc, axis=0, keepdims=True)

        cp_gw.wait()
        cp_b1.wait()
        cp_b2.wait()

        def flat(ref):
            return jnp.concatenate([ref[i:i + 1, :] for i in range(ref.shape[0])], axis=1).astype(f32)

        gate = jax.nn.sigmoid(jnp.sum(x_v[...].astype(f32) * flat(gw_v), axis=1, keepdims=True))
        cp_w1.wait()
        h = jnp.dot(x8, w1_v[...], preferred_element_type=f32) + flat(b1_v)
        h = jax.nn.gelu(h, approximate=True).astype(bf16)
        b = jnp.zeros((8, D), f32)
        for t in range(NP):
            cp_w2(t).wait()
            b = b + jnp.dot(h[:, t * W2R:(t + 1) * W2R], w2_v[t * W2R:(t + 1) * W2R, :],
                            preferred_element_type=f32)
        b = b[0:1, :] + flat(b2_v)
        o_ref[...] = (gate * a + (1.0 - gate) * b).astype(o_ref.dtype)

    scratch = [
        pltpu.VMEM((1, D), bf16),
        pltpu.VMEM((F // 128, 128), bf16),
        pltpu.VMEM((D // 128, 128), bf16),
        pltpu.VMEM((D // 128, 128), bf16),
        pltpu.VMEM((NG, D, GR), bf16),
        pltpu.VMEM((NG, GR, D), bf16),
        pltpu.VMEM((D, F), bf16),
        pltpu.VMEM((F, D), bf16),
        pltpu.VMEM((NBUF, RC, W), bf16),
        pltpu.VMEM((NC, G, RC), bf16),
        pltpu.VMEM((G, W), bf16),
        pltpu.SemaphoreType.DMA((4,)),
        pltpu.SemaphoreType.DMA((NG,)),
        pltpu.SemaphoreType.DMA((NG,)),
        pltpu.SemaphoreType.DMA(()),
        pltpu.SemaphoreType.DMA((NP,)),
        pltpu.SemaphoreType.DMA((NBUF,)),
    ]
    return kernel, scratch


@jax.jit
def pallas_gated_mix__sliding_block_cached__dense_activation_gelu__decode_kernel(
    A_x: jax.Array,
    A_k_cache: jax.Array,
    A_v_cache: jax.Array,
    A_wq: jax.Array,
    A_wo: jax.Array,
    B_x: jax.Array,
    B_w1: jax.Array,
    B_b1: jax.Array,
    B_w2: jax.Array,
    B_b2: jax.Array,
    gate_w: jax.Array,
):
    del B_x
    B, Sq, D = A_x.shape
    _, H, S, DH = A_k_cache.shape
    F = B_w1.shape[1]
    W = min(4096, max(256, S // 4))
    assert (B, Sq) == (1, 1) and H % _G == 0 and (_G * DH) % _RC == 0

    kernel, scratch = _make_kernel(H, DH, S, W, D, F)
    hbm = pl.BlockSpec(memory_space=pltpu.HBM)
    out = pl.pallas_call(
        kernel,
        out_shape=jax.ShapeDtypeStruct((1, D), A_x.dtype),
        in_specs=[hbm] * 10,
        out_specs=pl.BlockSpec(memory_space=pltpu.VMEM),
        scratch_shapes=scratch,
        compiler_params=pltpu.CompilerParams(vmem_limit_bytes=64 * 1024 * 1024),
    )(
        A_x.reshape(1, D),
        jnp.transpose(A_k_cache, (0, 1, 3, 2)).reshape(H * DH, S),
        jnp.transpose(A_v_cache, (0, 1, 3, 2)).reshape(H * DH, S),
        A_wq,
        A_wo,
        B_w1,
        B_b1.reshape(F // 128, 128),
        B_w2,
        B_b2.reshape(D // 128, 128),
        gate_w.reshape(D // 128, 128),
    )
    return out.reshape(1, 1, D)
```

```python
import jax
import jax.numpy as jnp
from jax import lax
from jax.experimental import pallas as pl
from jax.experimental.pallas import tpu as pltpu

_G = 8
_RC = 128
_LOOKAHEAD = 2
_W2_PIECES = 4
_KV_PIECE = (8, 1024)
_WIDE_PIECE = (8, 768)
_TALL_PIECE_ROWS = 16


def _make_kernel(H, DH, S, W, D, F):
    G, RC, L, NP = _G, _RC, _LOOKAHEAD, _W2_PIECES
    NG = H // G
    GR = G * DH
    NC = GR // RC
    NCH = NG * 2 * NC
    NBUF = L + 1
    W2R = F // NP
    f32, bf16 = jnp.float32, jnp.bfloat16
    sr, sc = _KV_PIECE
    kv_pieces = [(r, c) for c in range(0, W, sc) for r in range(0, RC, sr)]

    def kernel(x_hbm, k_hbm, v_hbm, wq_hbm, wo_hbm, w1_hbm, b1_hbm, w2_hbm, b2_hbm, gw_hbm,
               o_ref,
               x_v, b1_v, b2_v, gw_v, wq_v, wo_v, w1_v, w2_v, ring, qbd, p_v,
               sem_small, sem_wq, sem_wo, sem_w1, sem_w2, sem_ring):

        def start_split(src, r0, c0, dst, piece, sem):
            nrows, ncols = dst.shape
            pr, pc = piece

            def body(t, _):
                for u in range(2):
                    r = pl.multiple_of((2 * t + u) * pr, pr)
                    for ci, c in enumerate(range(0, ncols, pc)):
                        pltpu.make_async_copy(
                            src.at[pl.ds(r0 + r, pr), pl.ds(c0 + c, pc)],
                            dst.at[pl.ds(r, pr), pl.ds(c, pc)], sem,
                        ).start(priority=(u + ci) % 2)
                return 0

            lax.fori_loop(0, nrows // (2 * pr), body, 0)

        def wait_whole(dst, sem):
            pltpu.make_async_copy(dst, dst, sem).wait()

        tall = (_TALL_PIECE_ROWS, D)

        def start_wq(g):
            c0 = g * GR if isinstance(g, int) else pl.multiple_of(g * GR, GR)
            start_split(wq_hbm, 0, c0, wq_v.at[g], _WIDE_PIECE, sem_wq.at[g])

        def start_wo(g):
            start_split(wo_hbm, pl.multiple_of(g * GR, GR), 0, wo_v.at[g], tall, sem_wo.at[g])

        def start_ffn():
            start_split(w1_hbm, 0, 0, w1_v, _WIDE_PIECE, sem_w1)
            for t in range(NP):
                start_split(w2_hbm, t * W2R, 0, w2_v.at[t], tall, sem_w2.at[t])

        small = [
            pltpu.make_async_copy(src, dst, sem_small.at[i])
            for i, (src, dst) in enumerate(
                ((x_hbm, x_v), (gw_hbm, gw_v), (b1_hbm, b1_v), (b2_hbm, b2_v)))
        ]

        def start_chunk(src, row0, slot):
            for i, (r, c) in enumerate(kv_pieces):
                pltpu.make_async_copy(
                    src.at[pl.ds(row0 + r, sr), pl.ds(S - W + c, sc)],
                    ring.at[slot, pl.ds(r, sr), pl.ds(c, sc)], sem_ring.at[slot],
                ).start(priority=i % 2)

        def issue(j):
            g, r = j // (2 * NC), j % (2 * NC)
            is_v, c = r // NC, r % NC
            slot = j % NBUF
            if isinstance(j, int):
                start_chunk(v_hbm if is_v else k_hbm, g * GR + c * RC, slot)
            else:
                row0 = pl.multiple_of(g * GR + c * RC, RC)

                @pl.when(is_v == 0)
                def _():
                    start_chunk(k_hbm, row0, slot)

                @pl.when(is_v == 1)
                def _():
                    start_chunk(v_hbm, row0, slot)

        def advance(i):
            slot = i % NBUF
            wait_whole(ring.at[slot], sem_ring.at[slot])
            j = i + L

            @pl.when(j < NCH)
            def _():
                issue(j)

            @pl.when(j == NCH)
            def _():
                start_ffn()

            return slot

        small[0].start()
        start_wq(0)
        for j in range(L):
            issue(j)
        for cp in small[1:]:
            cp.start()
        small[0].wait()

        x8 = jnp.broadcast_to(x_v[...].astype(f32), (8, D)).astype(bf16)
        row = lax.broadcasted_iota(jnp.int32, (G, RC), 0)
        col = lax.broadcasted_iota(jnp.int32, (G, RC), 1)

        def own_head(c):
            return row == (c * RC + col) // DH

        def group(g, out_acc):
            start_wo(g)

            @pl.when(g + 1 < NG)
            def _():
                start_wq(g + 1)

            wait_whole(wq_v.at[g], sem_wq.at[g])
            q = jnp.dot(x8, wq_v[g], preferred_element_type=f32)
            for c in range(NC):
                qbd[c] = jnp.where(own_head(c), q[:, c * RC:(c + 1) * RC], 0.0).astype(bf16)

            def kstep(c, s):
                slot = advance(g * 2 * NC + c)
                return s + jnp.dot(qbd[c], ring[slot], preferred_element_type=f32)

            s = lax.fori_loop(0, NC, kstep, jnp.zeros((G, W), f32)) * (DH ** -0.5)
            p = jnp.exp(s - jnp.max(s, axis=1, keepdims=True))
            linv = 1.0 / jnp.sum(p, axis=1, keepdims=True)
            p_v[...] = p.astype(bf16)
            wait_whole(wo_v.at[g], sem_wo.at[g])

            def vstep(c, acc):
                slot = advance(g * 2 * NC + NC + c)
                o = lax.dot_general(p_v[...], ring[slot], (((1,), (1,)), ((), ())),
                                    preferred_element_type=f32)
                o = jnp.where(own_head(c), o * linv, 0.0).astype(bf16)
                r0 = pl.multiple_of(c * RC, RC)
                return acc + jnp.dot(o, wo_v[g, pl.ds(r0, RC), :], preferred_element_type=f32)

            return lax.fori_loop(0, NC, vstep, out_acc)

        out_acc = lax.fori_loop(0, NG, group, jnp.zeros((G, D), f32))
        a = jnp.sum(out_acc, axis=0, keepdims=True)

        for cp in small[1:]:
            cp.wait()

        def flat(ref):
            return jnp.concatenate([ref[i:i + 1, :] for i in range(ref.shape[0])], axis=1).astype(f32)

        gate = jax.nn.sigmoid(jnp.sum(x_v[...].astype(f32) * flat(gw_v), axis=1, keepdims=True))
        b2 = flat(b2_v)
        wait_whole(w1_v, sem_w1)
        h = jnp.dot(x8, w1_v[...], preferred_element_type=f32) + flat(b1_v)
        h = jax.nn.gelu(h, approximate=True).astype(bf16)
        b = jnp.zeros((8, D), f32)
        for t in range(NP):
            wait_whole(w2_v.at[t], sem_w2.at[t])
            b = b + jnp.dot(h[:, t * W2R:(t + 1) * W2R], w2_v[t], preferred_element_type=f32)
        b = b[0:1, :] + b2
        o_ref[...] = (gate * a + (1.0 - gate) * b).astype(o_ref.dtype)

    scratch = [
        pltpu.VMEM((1, D), bf16),
        pltpu.VMEM((F // 128, 128), bf16),
        pltpu.VMEM((D // 128, 128), bf16),
        pltpu.VMEM((D // 128, 128), bf16),
        pltpu.VMEM((NG, D, GR), bf16),
        pltpu.VMEM((NG, GR, D), bf16),
        pltpu.VMEM((D, F), bf16),
        pltpu.VMEM((NP, W2R, D), bf16),
        pltpu.VMEM((NBUF, RC, W), bf16),
        pltpu.VMEM((NC, G, RC), bf16),
        pltpu.VMEM((G, W), bf16),
        pltpu.SemaphoreType.DMA((4,)),
        pltpu.SemaphoreType.DMA((NG,)),
        pltpu.SemaphoreType.DMA((NG,)),
        pltpu.SemaphoreType.DMA(()),
        pltpu.SemaphoreType.DMA((NP,)),
        pltpu.SemaphoreType.DMA((NBUF,)),
    ]
    return kernel, scratch


@jax.jit
def pallas_gated_mix__sliding_block_cached__dense_activation_gelu__decode_kernel(
    A_x: jax.Array,
    A_k_cache: jax.Array,
    A_v_cache: jax.Array,
    A_wq: jax.Array,
    A_wo: jax.Array,
    B_x: jax.Array,
    B_w1: jax.Array,
    B_b1: jax.Array,
    B_w2: jax.Array,
    B_b2: jax.Array,
    gate_w: jax.Array,
):
    del B_x
    B, Sq, D = A_x.shape
    _, H, S, DH = A_k_cache.shape
    F = B_w1.shape[1]
    W = min(4096, max(256, S // 4))
    assert (B, Sq) == (1, 1) and H % _G == 0 and (_G * DH) % _RC == 0

    kernel, scratch = _make_kernel(H, DH, S, W, D, F)
    hbm = pl.BlockSpec(memory_space=pltpu.HBM)
    out = pl.pallas_call(
        kernel,
        out_shape=jax.ShapeDtypeStruct((1, D), A_x.dtype),
        in_specs=[hbm] * 10,
        out_specs=pl.BlockSpec(memory_space=pltpu.VMEM),
        scratch_shapes=scratch,
        compiler_params=pltpu.CompilerParams(vmem_limit_bytes=64 * 1024 * 1024),
    )(
        A_x.reshape(1, D),
        jnp.transpose(A_k_cache, (0, 1, 3, 2)).reshape(H * DH, S),
        jnp.transpose(A_v_cache, (0, 1, 3, 2)).reshape(H * DH, S),
        A_wq,
        A_wo,
        B_w1,
        B_b1.reshape(F // 128, 128),
        B_w2,
        B_b2.reshape(D // 128, 128),
        gate_w.reshape(D // 128, 128),
    )
    return out.reshape(1, 1, D)
```

```python
import jax
import jax.numpy as jnp
from jax import lax
from jax.experimental import pallas as pl
from jax.experimental.pallas import tpu as pltpu

_G = 8
_RC = 128
_LOOKAHEAD = 2
_KV_PIECE = (8, 1024)
_WQ_SPLIT = (8, 1024, 10)
_WO_SPLIT = (16, 640, 8)
_W1_SPLIT = (8, 768, 2)
_W2_SPLIT = (8, 640, 4)


def _make_kernel(H, DH, S, W, D, F):
    G, RC, L = _G, _RC, _LOOKAHEAD
    NG = H // G
    GR = G * DH
    NC = GR // RC
    NCH = NG * 2 * NC
    NBUF = L + 1
    f32, bf16 = jnp.float32, jnp.bfloat16
    sr, sc = _KV_PIECE
    kv_pieces = [(r, c) for c in range(0, W, sc) for r in range(0, RC, sr)]

    def kernel(x_hbm, k_hbm, v_hbm, wq_hbm, wo_hbm, w1_hbm, b1_hbm, w2_hbm, b2_hbm, gw_hbm,
               o_ref,
               x_v, b1_v, b2_v, gw_v, wq_v, wo_v, w1_v, w2_v, ring, qbd, p_v,
               sem_small, sem_w, sem_ring):

        def start_weight(src, dst, split, sem):
            nrows, ncols = dst.shape
            pr, pc, nbands = split
            band = nrows // nbands

            def body(t, _):
                for c in range(0, ncols, pc):
                    for b in range(nbands):
                        r = pl.multiple_of(b * band + t * pr, 8)
                        pltpu.make_async_copy(
                            src.at[pl.ds(r, pr), pl.ds(c, pc)],
                            dst.at[pl.ds(r, pr), pl.ds(c, pc)], sem,
                        ).start(priority=b % 2)
                return 0

            lax.fori_loop(0, band // pr, body, 0)

        def wait_whole(dst, sem):
            pltpu.make_async_copy(dst, dst, sem).wait()

        def start_chunk(src, row0, slot):
            for i, (r, c) in enumerate(kv_pieces):
                pltpu.make_async_copy(
                    src.at[pl.ds(row0 + r, sr), pl.ds(S - W + c, sc)],
                    ring.at[slot, pl.ds(r, sr), pl.ds(c, sc)], sem_ring.at[slot],
                ).start(priority=i % 2)

        def issue(j):
            g, r = j // (2 * NC), j % (2 * NC)
            is_v, c = r // NC, r % NC
            slot = j % NBUF
            if isinstance(j, int):
                start_chunk(v_hbm if is_v else k_hbm, g * GR + c * RC, slot)
            else:
                row0 = pl.multiple_of(g * GR + c * RC, RC)

                @pl.when(is_v == 0)
                def _():
                    start_chunk(k_hbm, row0, slot)

                @pl.when(is_v == 1)
                def _():
                    start_chunk(v_hbm, row0, slot)

        def advance(i):
            slot = i % NBUF
            wait_whole(ring.at[slot], sem_ring.at[slot])

            @pl.when(i + L < NCH)
            def _():
                issue(i + L)

            return slot

        def flat(ref):
            return jnp.concatenate([ref[i:i + 1, :] for i in range(ref.shape[0])], axis=1).astype(f32)

        small = [
            pltpu.make_async_copy(src, dst, sem_small.at[i])
            for i, (src, dst) in enumerate(
                ((x_hbm, x_v), (gw_hbm, gw_v), (b1_hbm, b1_v), (b2_hbm, b2_v)))
        ]

        for cp in small:
            cp.start()
        start_weight(w1_hbm, w1_v, _W1_SPLIT, sem_w.at[0])
        start_weight(w2_hbm, w2_v, _W2_SPLIT, sem_w.at[1])
        start_weight(wq_hbm, wq_v, _WQ_SPLIT, sem_w.at[2])
        for cp in small:
            cp.wait()
        x8 = jnp.broadcast_to(x_v[...].astype(f32), (G, D)).astype(bf16)
        wait_whole(w1_v, sem_w.at[0])
        h = jnp.dot(x8, w1_v[...], preferred_element_type=f32) + flat(b1_v)
        h = jax.nn.gelu(h, approximate=True).astype(bf16)
        start_weight(wo_hbm, wo_v, _WO_SPLIT, sem_w.at[3])
        wait_whole(w2_v, sem_w.at[1])
        ffn = jnp.dot(h, w2_v[...], preferred_element_type=f32)[0:1, :] + flat(b2_v)
        gate = jax.nn.sigmoid(jnp.sum(x_v[...].astype(f32) * flat(gw_v), axis=1, keepdims=True))
        ffn_mix = (1.0 - gate) * ffn
        for j in range(L):
            issue(j)
        wait_whole(wq_v, sem_w.at[2])

        row = lax.broadcasted_iota(jnp.int32, (G, RC), 0)
        col = lax.broadcasted_iota(jnp.int32, (G, RC), 1)

        def own_head(c, val):
            return jnp.where(row == (c * RC + col) // DH, val, 0.0).astype(bf16)

        q = jnp.dot(x8, wq_v[:, 0:GR], preferred_element_type=f32)
        for c in range(NC):
            qbd[0, c] = own_head(c, q[:, c * RC:(c + 1) * RC])

        def pv_wo(slot, row0, c, acc):
            o = lax.dot_general(p_v[...], ring[slot], (((1,), (1,)), ((), ())),
                                preferred_element_type=f32)
            return acc + jnp.dot(own_head(c, o), wo_v[pl.ds(row0, RC), :],
                                 preferred_element_type=f32)

        def group(g, out_acc):
            par = g % 2
            g_next = jnp.minimum(g + 1, NG - 1)

            def kstep(c, s):
                slot = advance(g * 2 * NC + c)
                s = s + jnp.dot(qbd[par, c], ring[slot], preferred_element_type=f32)
                c0 = pl.multiple_of(g_next * GR + c * RC, RC)
                qbd[1 - par, c] = own_head(
                    c, jnp.dot(x8, wq_v[:, pl.ds(c0, RC)], preferred_element_type=f32))
                return s

            s = lax.fori_loop(0, NC, kstep, jnp.zeros((G, W), f32)) * (DH ** -0.5)
            p = jnp.exp(s - jnp.max(s, axis=1, keepdims=True))
            p_v[...] = (p * (1.0 / jnp.sum(p, axis=1, keepdims=True))).astype(bf16)

            @pl.when(g == 0)
            def _():
                wait_whole(wo_v, sem_w.at[3])

            def vstep(c, acc):
                slot = advance(g * 2 * NC + NC + c)
                return pv_wo(slot, pl.multiple_of(g * GR + c * RC, RC), c, acc)

            return lax.fori_loop(0, NC, vstep, out_acc)

        out_acc = lax.fori_loop(0, NG, group, jnp.zeros((G, D), f32))
        attn = jnp.sum(out_acc, axis=0, keepdims=True)
        o_ref[...] = (gate * attn + ffn_mix).astype(o_ref.dtype)

    scratch = [
        pltpu.VMEM((1, D), bf16),
        pltpu.VMEM((F // 128, 128), bf16),
        pltpu.VMEM((D // 128, 128), bf16),
        pltpu.VMEM((D // 128, 128), bf16),
        pltpu.VMEM((D, H * DH), bf16),
        pltpu.VMEM((H * DH, D), bf16),
        pltpu.VMEM((D, F), bf16),
        pltpu.VMEM((F, D), bf16),
        pltpu.VMEM((NBUF, RC, W), bf16),
        pltpu.VMEM((2, NC, G, RC), bf16),
        pltpu.VMEM((G, W), bf16),
        pltpu.SemaphoreType.DMA((4,)),
        pltpu.SemaphoreType.DMA((4,)),
        pltpu.SemaphoreType.DMA((NBUF,)),
    ]
    return kernel, scratch


@jax.jit
def pallas_gated_mix__sliding_block_cached__dense_activation_gelu__decode_kernel(
    A_x: jax.Array,
    A_k_cache: jax.Array,
    A_v_cache: jax.Array,
    A_wq: jax.Array,
    A_wo: jax.Array,
    B_x: jax.Array,
    B_w1: jax.Array,
    B_b1: jax.Array,
    B_w2: jax.Array,
    B_b2: jax.Array,
    gate_w: jax.Array,
):
    del B_x
    B, Sq, D = A_x.shape
    _, H, S, DH = A_k_cache.shape
    F = B_w1.shape[1]
    W = min(4096, max(256, S // 4))
    assert (B, Sq) == (1, 1) and H % _G == 0 and (_G * DH) % _RC == 0

    kernel, scratch = _make_kernel(H, DH, S, W, D, F)
    hbm = pl.BlockSpec(memory_space=pltpu.HBM)
    out = pl.pallas_call(
        kernel,
        out_shape=jax.ShapeDtypeStruct((1, D), A_x.dtype),
        in_specs=[hbm] * 10,
        out_specs=pl.BlockSpec(memory_space=pltpu.VMEM),
        scratch_shapes=scratch,
        compiler_params=pltpu.CompilerParams(
            vmem_limit_bytes=64 * 1024 * 1024,
            disable_bounds_checks=True,
            disable_semaphore_checks=True,
        ),
    )(
        A_x.reshape(1, D),
        jnp.transpose(A_k_cache, (0, 1, 3, 2)).reshape(H * DH, S),
        jnp.transpose(A_v_cache, (0, 1, 3, 2)).reshape(H * DH, S),
        A_wq,
        A_wo,
        B_w1,
        B_b1.reshape(F // 128, 128),
        B_w2,
        B_b2.reshape(D // 128, 128),
        gate_w.reshape(D // 128, 128),
    )
    return out.reshape(1, 1, D)
```
